```python
import os as _os
_os.environ.setdefault("JAX_PLATFORMS", "cpu")
import jax
import jax.numpy as jnp

def _softmax(x, axis=-1):
    return jax.nn.softmax(x, axis=axis)
def _gelu(x):
    return jax.nn.gelu(x, approximate=True)
def _silu(x):
    return jax.nn.silu(x)
def _sigmoid(x):
    return jax.nn.sigmoid(x)
def _layernorm(x, axis=-1, eps=1e-5):
    m = jnp.mean(x, axis=axis, keepdims=True)
    v = jnp.var(x, axis=axis, keepdims=True)
    return (x - m) / jnp.sqrt(v + eps)
def _scatter_add(tgt, idx, src, axis=0):
    return tgt.at[idx].add(src)
def _segment_sum(src, seg, n):
    return jax.ops.segment_sum(src, seg, n)
class _Rng:
    def __init__(self, key):
        self._k = key
    def _next(self):
        self._k, sub = jax.random.split(self._k)
        return sub
    def normal(self, shape):
        return jax.random.normal(self._next(), shape, dtype=jnp.bfloat16)
    def randint(self, lo, hi, shape):
        return jax.random.randint(self._next(), shape, lo, hi, dtype=jnp.int32)
    def uniform(self, shape, lo=0.0, hi=1.0):
        return jax.random.uniform(self._next(), shape, jnp.bfloat16, lo, hi)
    def permutation(self, n):
        return jax.random.permutation(self._next(), n)


kernel_name = 'standalone__dcn_v2_cross__recsys'

def setup_inputs():
    _rng = _Rng(jax.random.key(int.from_bytes(__import__("os").urandom(4), "little")))
    _w = (lambda a: (lambda t: t.astype(jnp.bfloat16) if jnp.issubdtype(t.dtype, jnp.floating) else t)(jnp.asarray(a)))
    B, F, D, L = 4096, 26, 128, 6
    Din = min(F * D, 1024)
    return {
        "x0": _w((lambda *s: _rng.normal(s) * 0.05)(B, Din)),
        "ws": _w((lambda *s: _rng.normal(s) * 0.05)(L, Din, Din)),
        "bs": _w((lambda *s: _rng.normal(s) * 0.05)(L, Din)),
    }

def reference(x0, ws, bs):
    x = x0
    for l in range(ws.shape[0]):
        x = x0 * (x @ ws[l] + bs[l]) + x
    return x
```

```python
import contextlib
import jax, jax.numpy as jnp
from jax import lax
import jax.experimental.pallas as pl
import jax.experimental.pallas.tpu as pltpu

f32 = jnp.float32
bf16 = jnp.bfloat16

ORD_E = (3, 6, 5, 1, 2, 4, 7)
ORD_O = (4, 7, 2, 1, 5, 3, 6)
TIDX = {1: 0, 3: 1, 4: 2, 6: 3, 7: 4}
NEED = {(0, 0): (1, 4, 5, 7), (0, 1): (3, 5), (1, 0): (2, 4), (1, 1): (1, 2, 3, 6)}

def make(tm=512, scopes=False, ord_a=(2, 5, 1, 4, 7, 3, 6), last_split=4, l0_mode=1, ord_e=ORD_E, ord_o=ORD_O):
    H = 512
    hm = tm // 2
    L = 6
    B, D = 4096, 1024
    NT = B // tm
    scope = jax.named_scope if scopes else (lambda n: contextlib.nullcontext())

    def lhs(k, xq, xq_bf=None):
        a11, a12 = xq[0]
        a21, a22 = xq[1]
        if xq_bf is not None and k == 3:
            return xq_bf[0][0]
        if xq_bf is not None and k == 4:
            return xq_bf[1][1]
        return {1: lambda: a11 + a22, 2: lambda: a21 + a22, 3: lambda: a11, 4: lambda: a22,
                5: lambda: a11 + a12, 6: lambda: a21 - a11, 7: lambda: a12 - a22}[k]().astype(bf16)

    def cquad(m, r, c):
        if (r, c) == (0, 0):
            return m[1] + m[4] - m[5] + m[7]
        if (r, c) == (0, 1):
            return m[3] + m[5]
        if (r, c) == (1, 0):
            return m[2] + m[4]
        return m[1] - m[2] + m[3] + m[6]

    def combine(m, xq, x0q, bq):
        return [[x0q[r][c] * (cquad(m, r, c) + bq[c]) + xq[r][c] for c in range(2)] for r in range(2)]

    def kern(x0_hbm, w_hbm, b_hbm, o_hbm, x0_v, w_v, t_v, o_v, xs_v, b_v, bf_v,
             sem_x, sem_w, sem_o, sem_p, sem_r):
        def cp_x(i):
            return pltpu.make_async_copy(x0_hbm.at[pl.ds(i * tm, tm)], x0_v.at[pl.ds(i * tm, tm)], sem_x.at[0])
        cp_x_rest = pltpu.make_async_copy(x0_hbm.at[pl.ds(tm, B - tm)], x0_v.at[pl.ds(tm, B - tm)], sem_x.at[0])
        def cp_w(l):
            return pltpu.make_async_copy(w_hbm.at[l], w_v.at[l], sem_w.at[l - 1])
        def cp_xh(r, s):
            return pltpu.make_async_copy(x0_hbm.at[pl.ds(r * hm, hm)], x0_v.at[pl.ds(r * hm, hm)], sem_p.at[s])
        def cp_xq(r, c, s):
            return pltpu.make_async_copy(x0_hbm.at[pl.ds(r * hm, hm), pl.ds(c * H, H)],
                                         x0_v.at[pl.ds(r * hm, hm), pl.ds(c * H, H)], sem_p.at[s])
        def cp_wq(r, c, s):
            return pltpu.make_async_copy(w_hbm.at[0, pl.ds(r * H, H), pl.ds(c * H, H)],
                                         w_v.at[0, pl.ds(r * H, H), pl.ds(c * H, H)], sem_p.at[s])
        def cp_b(s):
            return pltpu.make_async_copy(b_hbm, b_v, sem_p.at[s])
        def cp_o(row, nrow, col, ncol):
            return pltpu.make_async_copy(o_v.at[pl.ds(row, nrow), pl.ds(col, ncol)],
                                         o_hbm.at[pl.ds(row, nrow), pl.ds(col, ncol)], sem_o.at[0])
        cp_o_all = pltpu.make_async_copy(o_v, o_hbm, sem_o.at[0])

        def fence():
            pl.semaphore_signal(sem_r, 1)
            pl.semaphore_wait(sem_r, 1)

        def wq(l, r, c):
            return w_v[l, r * H:(r + 1) * H, c * H:(c + 1) * H]

        def rhs_fly(l, k):
            if k == 2:
                return wq(l, 0, 0)
            if k == 5:
                return wq(l, 1, 1)
            (p, q, sgn) = {1: ((0, 0), (1, 1), 1), 3: ((0, 1), (1, 1), -1), 4: ((1, 0), (0, 0), -1),
                           6: ((0, 0), (0, 1), 1), 7: ((1, 0), (1, 1), 1)}[k]
            u = wq(l, *p).astype(f32)
            v = wq(l, *q).astype(f32)
            t = (u + v if sgn > 0 else u - v).astype(bf16)
            t_v[l, TIDX[k]] = t
            return t

        def rhs(l, k):
            if k == 2:
                return wq(l, 0, 0)
            if k == 5:
                return wq(l, 1, 1)
            return t_v[l, TIDX[k]]

        def ld_x0(base=0):
            return [[x0_v[pl.ds(base + r * hm, hm), c * H:(c + 1) * H] for c in range(2)] for r in range(2)]

        def store_q(r, c, v):
            xs_v[r * hm:(r + 1) * hm, c * H:(c + 1) * H] = v
            o_v[r * hm:(r + 1) * hm, c * H:(c + 1) * H] = v.astype(bf16)

        if l0_mode == 0:
            groups = [([cp_xh(1, 0), cp_wq(0, 0, 0), cp_b(0)], (2,)),
                      ([cp_wq(1, 0, 1)], (4,)),
                      ([cp_xh(0, 2), cp_wq(1, 1, 2)], (5, 1, 7)),
                      ([cp_wq(0, 1, 3)], (3, 6))]
        elif l0_mode == 1:
            groups = [([cp_xh(1, 0), cp_wq(0, 0, 0), cp_b(0)], (2,)),
                      ([cp_wq(1, 0, 1)], (4,)),
                      ([cp_wq(1, 1, 2), cp_xq(0, 1, 2)], (7,)),
                      ([cp_xq(0, 0, 3)], (5, 1)),
                      ([cp_wq(0, 1, 4)], (3, 6))]
        elif l0_mode == 2:
            groups = [([cp_xh(1, 0), cp_wq(0, 0, 0), cp_b(0)], (2,)),
                      ([cp_wq(1, 0, 1)], (4,)),
                      ([cp_wq(1, 1, 2), cp_xq(0, 1, 2)], (7,)),
                      ([cp_xq(0, 0, 3), cp_wq(0, 1, 3)], (5, 1, 3, 6))]

        with scope("pro"):
            seq = [cp for g, _ in groups for cp in g]
            seq += [cp_w(l) for l in range(1, L)] + [cp_x_rest]
            for cp in seq:
                cp.start()
                fence()

        with scope("layer0"):
            m = {}
            def q(r, c):
                return x0_v[r * hm:(r + 1) * hm, c * H:(c + 1) * H]
            def qf(r, c):
                return q(r, c).astype(f32)
            lhs0 = {1: lambda: (qf(0, 0) + qf(1, 1)).astype(bf16), 2: lambda: (qf(1, 0) + qf(1, 1)).astype(bf16),
                    3: lambda: q(0, 0), 4: lambda: q(1, 1), 5: lambda: (qf(0, 0) + qf(0, 1)).astype(bf16),
                    6: lambda: (qf(1, 0) - qf(0, 0)).astype(bf16), 7: lambda: (qf(0, 1) - qf(1, 1)).astype(bf16)}
            done = set()
            for gi, (g, prods) in enumerate(groups):
                for cp in g:
                    cp.wait()
                if gi == 0:
                    for l in range(L):
                        bf_v[l] = b_v[l:l + 1, :].astype(f32)
                for k in prods:
                    m[k] = jnp.dot(lhs0[k](), rhs_fly(0, k), preferred_element_type=f32)
                    for (r, c), need in NEED.items():
                        if (r, c) not in done and all(n in m for n in need):
                            done.add((r, c))
                            x0f = qf(r, c)
                            store_q(r, c, x0f * (cquad(m, r, c) + bf_v[0, :, c * H:(c + 1) * H]) + x0f)

        def phase_a(l, carry):
            with scope("wait_w"):
                cp_w(l).wait()
            xq = [[xs_v[r * hm:(r + 1) * hm, c * H:(c + 1) * H] for c in range(2)] for r in range(2)]
            m = {}
            for k in ord_a:
                m[k] = jnp.dot(lhs(k, xq), rhs_fly(l, k), preferred_element_type=f32)
            x0q = [[x.astype(f32) for x in row] for row in ld_x0()]
            bq = [bf_v[l, :, c * H:(c + 1) * H] for c in range(2)]
            xn = combine(m, xq, x0q, bq)
            for r in range(2):
                for c in range(2):
                    store_q(r, c, xn[r][c])
            return carry
        with scope("phaseA"):
            lax.fori_loop(1, L, phase_a, 0)
        cp_o(0, tm, 0, D).start()
        cp_x_rest.wait()

        def phase_b(i, carry):
            base = pl.multiple_of(i * tm, tm)
            x0b = ld_x0(base)
            x0q = [[x0b[r][c].astype(f32) for c in range(2)] for r in range(2)]
            xq = x0q
            for l in range(L):
                bq = [bf_v[l, :, c * H:(c + 1) * H] for c in range(2)]
                m = {}
                for k in (ord_e if l % 2 == 0 else ord_o):
                    m[k] = jnp.dot(lhs(k, xq, x0b if l == 0 else None), rhs(l, k), preferred_element_type=f32)
                xq = combine(m, xq, x0q, bq)
            order = sorted(NEED, key=lambda rc: max(ord_o.index(n) for n in NEED[rc]))
            for j, (r, c) in enumerate(order):
                ns = last_split if j == 3 else 1
                w = H // ns
                for s in range(ns):
                    o_v[pl.ds(base + r * hm, hm), c * H + s * w:c * H + (s + 1) * w] = xq[r][c][:, s * w:(s + 1) * w].astype(bf16)
                    cp_o(base + r * hm, hm, c * H + s * w, w).start()
            return carry
        with scope("phaseB"):
            lax.fori_loop(1, NT, phase_b, 0)
        with scope("drain"):
            cp_o_all.wait()

    @jax.jit
    def f(x0, ws, bs):
        return pl.pallas_call(
            kern,
            in_specs=[pl.BlockSpec(memory_space=pl.ANY)] * 3,
            out_specs=pl.BlockSpec(memory_space=pl.ANY),
            out_shape=jax.ShapeDtypeStruct((B, D), x0.dtype),
            scratch_shapes=[
                pltpu.VMEM((B, D), bf16),
                pltpu.VMEM((L, D, D), bf16),
                pltpu.VMEM((L, 5, H, H), bf16),
                pltpu.VMEM((B, D), bf16),
                pltpu.VMEM((tm, D), f32),
                pltpu.VMEM((L, D), bf16),
                pltpu.VMEM((L, 1, D), f32),
                pltpu.SemaphoreType.DMA((1,)),
                pltpu.SemaphoreType.DMA((L - 1,)),
                pltpu.SemaphoreType.DMA((1,)),
                pltpu.SemaphoreType.DMA((5,)),
                pltpu.SemaphoreType.REGULAR,
            ],
            compiler_params=pltpu.CompilerParams(vmem_limit_bytes=110 * 1024 * 1024),
        )(x0, ws, bs)
    return f


_impl = make(l0_mode=2)


@jax.jit
def pallas_standalone__dcn_v2_cross__recsys_kernel(x0: jax.Array, ws: jax.Array, bs: jax.Array):
    return _impl(x0, ws, bs)
```

```python
import jax
import jax.numpy as jnp
from jax import lax
import jax.experimental.pallas as pl
import jax.experimental.pallas.tpu as pltpu

f32 = jnp.float32
bf16 = jnp.bfloat16

TM = 512

_WSUM = {1: ((0, 0), (1, 1), 1), 3: ((0, 1), (1, 1), -1), 4: ((1, 0), (0, 0), -1),
         6: ((0, 0), (0, 1), 1), 7: ((1, 0), (1, 1), 1)}
_WSLOT = {1: 0, 3: 1, 4: 2, 6: 3, 7: 4}
_NEED = {(0, 0): (1, 4, 5, 7), (0, 1): (3, 5), (1, 0): (2, 4), (1, 1): (1, 2, 3, 6)}
_ORD_EVEN = (3, 5, 4, 6, 2, 1, 7)
_ORD_ODD = (4, 2, 3, 7, 5, 1, 6)
_ORD_TILE0 = (2, 5, 1, 4, 7, 3, 6)
_LAST_SPLIT = 4


def _lhs(k, xq):
    (a11, a12), (a21, a22) = xq
    if k == 1:
        s = a11 + a22
    elif k == 2:
        s = a21 + a22
    elif k == 3:
        s = a11
    elif k == 4:
        s = a22
    elif k == 5:
        s = a11 + a12
    elif k == 6:
        s = a21 - a11
    else:
        s = a12 - a22
    return s.astype(bf16)


def _cquad(m, r, c):
    if (r, c) == (0, 0):
        return m[1] + m[4] - m[5] + m[7]
    if (r, c) == (0, 1):
        return m[3] + m[5]
    if (r, c) == (1, 0):
        return m[2] + m[4]
    return m[1] - m[2] + m[3] + m[6]


def _dot(a, b):
    return jnp.dot(a, b, preferred_element_type=f32)


def _kernel(x0_hbm, w_hbm, b_hbm, o_hbm,
            x0_v, w_v, t_v, o_v, xs_v, b_v, bf_v,
            sem_x, sem_w, sem_o, sem_p, sem_f):
    B, D = x0_v.shape
    L = w_v.shape[0]
    H = D // 2
    hm = TM // 2
    n_tiles = B // TM

    def cp_x0(r0, nr, c0, nc, s):
        return pltpu.make_async_copy(x0_hbm.at[pl.ds(r0, nr), pl.ds(c0, nc)],
                                     x0_v.at[pl.ds(r0, nr), pl.ds(c0, nc)], sem_p.at[s])

    def cp_w0(r, c, s):
        return pltpu.make_async_copy(w_hbm.at[0, pl.ds(r * H, H), pl.ds(c * H, H)],
                                     w_v.at[0, pl.ds(r * H, H), pl.ds(c * H, H)], sem_p.at[s])

    def cp_w(l):
        return pltpu.make_async_copy(w_hbm.at[l], w_v.at[l], sem_w.at[l - 1])

    def cp_o(r0, nr, c0, nc):
        return pltpu.make_async_copy(o_v.at[pl.ds(r0, nr), pl.ds(c0, nc)],
                                     o_hbm.at[pl.ds(r0, nr), pl.ds(c0, nc)], sem_o.at[0])

    cp_b = pltpu.make_async_copy(b_hbm, b_v, sem_p.at[0])
    cp_x_rest = pltpu.make_async_copy(x0_hbm.at[pl.ds(TM, B - TM)],
                                      x0_v.at[pl.ds(TM, B - TM)], sem_x.at[0])

    def wq(l, r, c):
        return w_v[l, r * H:(r + 1) * H, c * H:(c + 1) * H]

    def rhs_build(l, k):
        if k == 2:
            return wq(l, 0, 0)
        if k == 5:
            return wq(l, 1, 1)
        p, q, sgn = _WSUM[k]
        u = wq(l, *p).astype(f32)
        v = wq(l, *q).astype(f32)
        t = (u + v if sgn > 0 else u - v).astype(bf16)
        t_v[l, _WSLOT[k]] = t
        return t

    def rhs(l, k):
        if k == 2:
            return wq(l, 0, 0)
        if k == 5:
            return wq(l, 1, 1)
        return t_v[l, _WSLOT[k]]

    def bias(l, c):
        return bf_v[l, :, c * H:(c + 1) * H]

    def x0_quads(base):
        return [[x0_v[pl.ds(base + r * hm, hm), c * H:(c + 1) * H] for c in range(2)]
                for r in range(2)]

    def store_tile0(r, c, v):
        xs_v[r * hm:(r + 1) * hm, c * H:(c + 1) * H] = v
        o_v[r * hm:(r + 1) * hm, c * H:(c + 1) * H] = v.astype(bf16)

    groups = [
        ([cp_x0(hm, hm, 0, D, 0), cp_w0(0, 0, 0), cp_b], (2,)),
        ([cp_w0(1, 0, 1)], (4,)),
        ([cp_w0(1, 1, 2), cp_x0(0, hm, H, H, 2)], (7,)),
        ([cp_x0(0, hm, 0, H, 3), cp_w0(0, 1, 3)], (5, 1, 3, 6)),
    ]
    seq = [cp for g, _ in groups for cp in g]
    seq += [cp_w(l) for l in range(1, L)] + [cp_x_rest]
    for cp in seq:
        cp.start()
        pl.semaphore_signal(sem_f, 1)
        pl.semaphore_wait(sem_f, 1)

    def q0(r, c):
        return x0_v[r * hm:(r + 1) * hm, c * H:(c + 1) * H]

    def q0f(r, c):
        return q0(r, c).astype(f32)

    lhs0 = {
        1: lambda: (q0f(0, 0) + q0f(1, 1)).astype(bf16),
        2: lambda: (q0f(1, 0) + q0f(1, 1)).astype(bf16),
        3: lambda: q0(0, 0),
        4: lambda: q0(1, 1),
        5: lambda: (q0f(0, 0) + q0f(0, 1)).astype(bf16),
        6: lambda: (q0f(1, 0) - q0f(0, 0)).astype(bf16),
        7: lambda: (q0f(0, 1) - q0f(1, 1)).astype(bf16),
    }
    m = {}
    done = set()
    for gi, (g, prods) in enumerate(groups):
        for cp in g:
            cp.wait()
        if gi == 0:
            for l in range(L):
                bf_v[l] = b_v[l:l + 1, :].astype(f32)
        for k in prods:
            m[k] = _dot(lhs0[k](), rhs_build(0, k))
            for (r, c), need in _NEED.items():
                if (r, c) not in done and all(n in m for n in need):
                    done.add((r, c))
                    x0f = q0f(r, c)
                    store_tile0(r, c, x0f * (_cquad(m, r, c) + bias(0, c)) + x0f)

    def tile0_layer(l, carry):
        cp_w(l).wait()
        xq = [[xs_v[r * hm:(r + 1) * hm, c * H:(c + 1) * H] for c in range(2)]
              for r in range(2)]
        mm = {}
        for k in _ORD_TILE0:
            mm[k] = _dot(_lhs(k, xq), rhs_build(l, k))
        x0b = x0_quads(0)
        xn = [[x0b[r][c].astype(f32) * (_cquad(mm, r, c) + bias(l, c)) + xq[r][c]
               for c in range(2)] for r in range(2)]
        for r in range(2):
            for c in range(2):
                store_tile0(r, c, xn[r][c])
        return carry

    lax.fori_loop(1, L, tile0_layer, 0)
    cp_o(0, TM, 0, D).start()
    cp_x_rest.wait()

    last_ord = _ORD_EVEN if (L - 1) % 2 == 0 else _ORD_ODD
    out_order = sorted(_NEED, key=lambda rc: max(last_ord.index(n) for n in _NEED[rc]))

    def tile(i, carry):
        base = pl.multiple_of(i * TM, TM)
        x0b = x0_quads(base)
        x0q = [[x0b[r][c].astype(f32) for c in range(2)] for r in range(2)]
        xq = x0q
        for l in range(L):
            mm = {}
            for k in (_ORD_EVEN if l % 2 == 0 else _ORD_ODD):
                if l == 0 and k == 3:
                    a = x0b[0][0]
                elif l == 0 and k == 4:
                    a = x0b[1][1]
                else:
                    a = _lhs(k, xq)
                mm[k] = _dot(a, rhs(l, k))
            xq = [[x0q[r][c] * (_cquad(mm, r, c) + bias(l, c)) + xq[r][c]
                   for c in range(2)] for r in range(2)]
        for j, (r, c) in enumerate(out_order):
            ns = _LAST_SPLIT if j == len(out_order) - 1 else 1
            w = H // ns
            for s in range(ns):
                c0 = c * H + s * w
                o_v[pl.ds(base + r * hm, hm), c0:c0 + w] = (
                    xq[r][c][:, s * w:(s + 1) * w].astype(bf16))
                cp_o(base + r * hm, hm, c0, w).start()
        return carry

    lax.fori_loop(1, n_tiles, tile, 0)
    pltpu.make_async_copy(o_v, o_hbm, sem_o.at[0]).wait()


@jax.jit
def pallas_standalone__dcn_v2_cross__recsys_kernel(
    x0: jax.Array,
    ws: jax.Array,
    bs: jax.Array,
):
    B, D = x0.shape
    L = ws.shape[0]
    assert ws.shape == (L, D, D) and bs.shape == (L, D)
    assert B % TM == 0 and B > TM and L >= 2
    assert D % (256 * _LAST_SPLIT) == 0
    H = D // 2
    return pl.pallas_call(
        _kernel,
        in_specs=[pl.BlockSpec(memory_space=pl.ANY)] * 3,
        out_specs=pl.BlockSpec(memory_space=pl.ANY),
        out_shape=jax.ShapeDtypeStruct((B, D), x0.dtype),
        scratch_shapes=[
            pltpu.VMEM((B, D), bf16),
            pltpu.VMEM((L, D, D), bf16),
            pltpu.VMEM((L, 5, H, H), bf16),
            pltpu.VMEM((B, D), bf16),
            pltpu.VMEM((TM, D), f32),
            pltpu.VMEM((L, D), bf16),
            pltpu.VMEM((L, 1, D), f32),
            pltpu.SemaphoreType.DMA((1,)),
            pltpu.SemaphoreType.DMA((L - 1,)),
            pltpu.SemaphoreType.DMA((1,)),
            pltpu.SemaphoreType.DMA((4,)),
            pltpu.SemaphoreType.REGULAR,
        ],
        compiler_params=pltpu.CompilerParams(
            vmem_limit_bytes=100 * 1024 * 1024,
            disable_bounds_checks=True,
            disable_semaphore_checks=True,
        ),
    )(x0, ws, bs)
```
